```python
import os as _os
_os.environ.setdefault("JAX_PLATFORMS", "cpu")
import jax
import jax.numpy as jnp

def _softmax(x, axis=-1):
    return jax.nn.softmax(x, axis=axis)
def _gelu(x):
    return jax.nn.gelu(x, approximate=True)
def _silu(x):
    return jax.nn.silu(x)
def _sigmoid(x):
    return jax.nn.sigmoid(x)
def _layernorm(x, axis=-1, eps=1e-5):
    m = jnp.mean(x, axis=axis, keepdims=True)
    v = jnp.var(x, axis=axis, keepdims=True)
    return (x - m) / jnp.sqrt(v + eps)
def _scatter_add(tgt, idx, src, axis=0):
    return tgt.at[idx].add(src)
def _segment_sum(src, seg, n):
    return jax.ops.segment_sum(src, seg, n)
class _Rng:
    def __init__(self, key):
        self._k = key
    def _next(self):
        self._k, sub = jax.random.split(self._k)
        return sub
    def normal(self, shape):
        return jax.random.normal(self._next(), shape, dtype=jnp.bfloat16)
    def randint(self, lo, hi, shape):
        return jax.random.randint(self._next(), shape, lo, hi, dtype=jnp.int32)
    def uniform(self, shape, lo=0.0, hi=1.0):
        return jax.random.uniform(self._next(), shape, jnp.bfloat16, lo, hi)
    def permutation(self, n):
        return jax.random.permutation(self._next(), n)


kernel_name = 'concat_heads__sliding_local_dilated__sliding_block__prompt'

def setup_inputs():
    _rng = _Rng(jax.random.key(int.from_bytes(__import__("os").urandom(4), "little")))
    _w = (lambda a: (lambda t: t.astype(jnp.bfloat16) if jnp.issubdtype(t.dtype, jnp.floating) else t)(jnp.asarray(a)))
    def _A_setup():
        B, S, D = 1, 2048, 1024
        return {
            "x": _w((lambda *s: _rng.normal(s) * 0.2)(B, S, D)),
            "wqkv": _w((lambda *s: _rng.normal(s) * 0.2)(D, 3 * D)),
            "wo": _w((lambda *s: _rng.normal(s) * 0.05)(D, D)),
        }
    _A_in = _A_setup()

    def _B_setup():
        B, S, D = 1, 2048, 1024
        return {
            "x": _w((lambda *s: _rng.normal(s) * 0.2)(B, S, D)),
            "wqkv": _w((lambda *s: _rng.normal(s) * 0.2)(D, 3 * D)),
            "wo": _w((lambda *s: _rng.normal(s) * 0.05)(D, D)),
        }
    _B_in = _B_setup()

    return {
        "A_x": _A_in["x"],
        "A_wqkv": _A_in["wqkv"],
        "A_wo": _A_in["wo"],
        "B_x": _B_in["x"],
        "B_wqkv": _B_in["wqkv"],
        "B_wo": _B_in["wo"],
    }

def reference(A_x, A_wqkv, A_wo, B_x, B_wqkv, B_wo):
    def _A_ref(x, wqkv, wo):
        B, S, D = x.shape
        H = 32; Dh = D // H
        W, dil = 8, 2
        qkv = (lambda x, *d: x.transpose(*d))((x @ wqkv).reshape(B, S, 3, H, Dh), 2, 0, 3, 1, 4)
        q, k, v = qkv[0], qkv[1], qkv[2]
        scale = Dh ** -0.5
        pos = jnp.arange(S)
        off = jnp.arange(W) * dil
        idx = pos[:, None] - off[None, :]
        mask = idx >= 0
        idx_c = jnp.where(mask, idx, 0).reshape(-1)
        kg = k[:, :, idx_c, :].reshape(B, H, S, W, Dh)
        vg = v[:, :, idx_c, :].reshape(B, H, S, W, Dh)
        logits = jnp.einsum("bhsd,bhswd->bhsw", q, kg) * scale
        logits = jnp.where(mask[None, None, :, :], logits, -1e9)
        attn = _softmax(logits, axis=-1)
        o = jnp.einsum("bhsw,bhswd->bhsd", attn, vg)
        return (lambda x, *d: x.transpose(*d))(o, 0, 2, 1, 3).reshape(B, S, D) @ wo

    def _B_ref(x, wqkv, wo):
        B, S, D = x.shape
        H = 32; Dh = D // H; W = 256
        qkv = (lambda x, *d: x.transpose(*d))((x @ wqkv).reshape(B, S, 3, H, Dh), 2, 0, 3, 1, 4)
        q, k, v = qkv[0], qkv[1], qkv[2]
        scores = jnp.einsum("bhqd,bhkd->bhqk", q, k) * (Dh ** -0.5)
        idx = jnp.arange(S)
        mask = (idx[:, None] - idx[None, :] >= 0) & (idx[:, None] - idx[None, :] < W)
        scores = jnp.where(mask[None, None], scores, -1e9)
        p = _softmax(scores, axis=-1)
        o = jnp.einsum("bhqk,bhkd->bhqd", p, v)
        return (lambda x, *d: x.transpose(*d))(o, 0, 2, 1, 3).reshape(B, S, D) @ wo

    a = _A_ref(A_x, A_wqkv, A_wo)
    b = _B_ref(B_x, B_wqkv, B_wo)
    return jnp.concatenate([a, b], axis=-1)
```

```python
import functools
import math

import numpy as np
import jax
import jax.numpy as jnp
from jax import lax
from jax.experimental import pallas as pl
from jax.experimental.pallas import tpu as pltpu

S, D = 2048, 1024
H, DH = 32, 32
PAD = 256
NEG = -1e30
CQ = float(DH ** -0.5 * math.log2(math.e))
bf16, f32, u32, i32 = jnp.bfloat16, jnp.float32, jnp.uint32, jnp.int32


def u2b(x):
    return pltpu.bitcast(x, bf16)


def b2u(x):
    return pltpu.bitcast(x, u32)


def packi(p):
    n = p.shape[0]
    return jnp.concatenate(
        [pltpu.pack_elementwise([p[16 * j:16 * j + 8], p[16 * j + 8:16 * j + 16]], packed_dtype=bf16)
         for j in range(n // 16)], axis=0)


def mo(x, m):
    return pl.multiple_of(x, m)


class Attn:
    def __init__(self, rows, win0, vwin0, vwidth):
        self.R = rows
        self.win0 = win0
        self.vwin0 = vwin0
        self.vwidth = vwidth
        self.NS = rows // 16
        self.NT = self.NS + 6
        self.lead = (win0 - vwin0) // 16


ATT_B = Attn(288, -256, -256, 384)
ATT_A = Attn(48, -16, -128, 256)


def build(RB=256, RB0=512, order="inter2", early="sel", opw=256, unroll=1, nbuf=2, debug=False):
    NB = S // RB

    def qkv_piece(X, W, r0, nrows, n, Q32, K32, VT32, wcol0=0):
        x = X[pl.ds(mo(r0, 16), nrows), :]
        c0 = n * 128 - wcol0
        r = jnp.dot(x, W[:, c0:c0 + 128], preferred_element_type=f32)
        g = n % 8
        lanes = slice(g * 128, (g + 1) * 128)
        if n < 8:
            Q32.bitcast(bf16)[pl.ds(mo(r0, 16), nrows), lanes] = (r * CQ).astype(bf16)
        elif n < 16:
            K32.bitcast(bf16)[pl.ds(mo(r0 + PAD, 16), nrows), lanes] = r.astype(bf16)
        else:
            vt = u2b(packi(r)).T
            VT32.bitcast(bf16)[lanes, pl.ds(mo(r0 + PAD, 128), nrows)] = vt

    def out_piece(O32, WO, OUT, r0, nrows, n, col0):
        o = u2b(O32[pl.ds(mo(r0 // 2, 8), nrows // 2), :])
        r = jnp.dot(o, WO[:, n * opw:(n + 1) * opw], preferred_element_type=f32)
        OUT[pl.ds(mo(r0, 16), nrows), col0 + n * opw:col0 + (n + 1) * opw] = r.astype(bf16)

    def qk_unit(att, Q32, K32, bias, Sb, Mb, q32, q0, g, s, off):
        lanes = slice(g * 128, (g + 1) * 128)
        lane = lax.broadcasted_iota(i32, (16, 128), 1)
        Qblk = Q32[pl.ds(mo(q32 + 16 * s, 8), 16), lanes]
        zero = jnp.zeros((16, 128), u32)
        Qm = u2b(jnp.concatenate([jnp.where(lane // 32 == h, Qblk, zero) for h in range(4)], axis=0))
        k32 = q32 + (PAD + 32 * s + att.win0) // 2
        Kw = u2b(K32[pl.ds(mo(k32, 8), att.R // 2), lanes])
        St = lax.dot_general(Kw, Qm, (((1,), (1,)), ((), ())), preferred_element_type=f32)
        pieces = []
        if att is ATT_B:
            kpos = q0 + 32 * s - 256
            for i8 in range(9):
                x = St[32 * i8:32 * i8 + 32]
                if i8 == 0:
                    x = x + bias[0:32, :]
                elif i8 == 8:
                    x = x + bias[32:64, :]
                if i8 < 8 and early == "sel":
                    x = jnp.where(kpos + 32 * i8 >= 0, x, NEG)
                pieces.append((32 * i8, x))
        else:
            x0 = St[0:16] + bias[0:16, :]
            if s == 0 and early == "sel":
                x0 = jnp.where(q0 > 0, x0, NEG)
            pieces.append((0, x0))
            pieces.append((16, St[16:48] + bias[16:48, :]))
        mx = None
        for (r0, x) in pieces:
            n = x.shape[0]
            Sb[pl.ds(mo(off + r0, 8), n), s * 128:(s + 1) * 128] = x
            y = jnp.max(x.reshape(n // 8, 8, 128), axis=0)
            mx = y if mx is None else jnp.maximum(mx, y)
        Mb[:, s * 128:(s + 1) * 128] = jnp.broadcast_to(jnp.max(mx, axis=0, keepdims=True), (8, 128))

    def smpv_parts(att, VT32, O32, Sb, Mb, q0, g, off):
        st = {"l": [None] * 4, "T": [[None] * att.NT for _ in range(4)]}
        lane8 = lax.broadcasted_iota(i32, (8, 128), 1)

        def blk(s):
            return lane8 // 32 == s

        def do_a(a):
            rots = {}
            for s in range(4):
                src = a - 2 * s
                if 0 <= src < att.NS:
                    m = Mb[:, s * 128:(s + 1) * 128]
                    x = Sb[pl.ds(mo(off + 16 * src, 8), 16), s * 128:(s + 1) * 128]
                    p0 = jnp.exp2(x[0:8] - m)
                    p1 = jnp.exp2(x[8:16] - m)
                    ps = p0 + p1
                    st["l"][s] = ps if st["l"][s] is None else st["l"][s] + ps
                    pu = pltpu.pack_elementwise([p0, p1], packed_dtype=bf16)
                    rots[s] = [pu] + [pltpu.roll(pu, 32 * t, axis=1) for t in (1, 2, 3)]
            for h in range(4):
                cur = None
                for s in rots:
                    v = rots[s][(s - h) % 4]
                    cur = jnp.where(blk(s), v, jnp.zeros((8, 128), u32) if cur is None else cur)
                st["T"][h][a] = cur

        def finish():
            lred = []
            for s in range(4):
                ls = jnp.broadcast_to(jnp.sum(st["l"][s], axis=0, keepdims=True), (8, 128))
                lred.append([ls] + [pltpu.roll(ls, 32 * t, axis=1) for t in (1, 2, 3)])
            ots = []
            for h in range(4):
                tl = [jnp.zeros((8, 128), u32)] * att.lead + st["T"][h]
                Th = u2b(jnp.concatenate(tl, axis=0))
                f32row = (g * 128 + h * 32) // 2
                Vt = u2b(VT32[f32row:f32row + 16, pl.ds(mo(q0 + PAD + att.vwin0, 128), att.vwidth)])
                ot = jnp.dot(Vt, Th, preferred_element_type=f32)
                lh = None
                for s in range(4):
                    v = lred[s][(s - h) % 4]
                    lh = v if lh is None else jnp.where(blk(s), v, lh)
                inv = 1.0 / lh
                ots.append(ot * jnp.concatenate([inv] * 4, axis=0))
            OTg = jnp.concatenate(ots, axis=0).astype(bf16)
            O32.bitcast(bf16)[pl.ds(mo(q0, 128), 128), g * 128:(g + 1) * 128] = OTg.T

        nt = att.NT
        bounds = [(nt * k) // 4 for k in range(5)]

        def part(k):
            for a in range(bounds[k], bounds[k + 1]):
                do_a(a)
            if k == 3:
                finish()
        return [functools.partial(part, k) for k in range(4)]

    def attn_loop(att, Q32, K32, VT32, O32, bias, Sbufs, Mbufs, fillers_fn, pre_fn=None, post_fn=None):
        nqb = RB // 128
        steps = [(qb, g) for qb in range(nqb) for g in range(8)]
        ns = len(steps)

        def qk_parts(i, t, offw):
            if t == ns:
                i2 = jnp.minimum(i + 1, NB - 1)
                qb, g = steps[0]
            else:
                i2 = i
                qb, g = steps[t]
            q32 = i2 * (RB // 2) + 64 * qb
            q0 = i2 * RB + 128 * qb
            slot = t % nbuf
            return [functools.partial(qk_unit, att, Q32, K32, bias, Sbufs[slot], Mbufs[slot], q32, q0, g, s, offw)
                    for s in range(4)]

        for f in qk_parts(0, 0, 0):
            f()

        def body(i, c):
            offw = i >> 8
            offr = i >> 9
            if pre_fn is not None:
                pre_fn(i)
            fl = fillers_fn(i)
            nf = len(fl)
            per = [fl[(nf * t) // ns:(nf * (t + 1)) // ns] for t in range(ns)]
            for t in range(ns):
                a = qk_parts(i, t + 1, offw)
                qb, g = steps[t]
                b = smpv_parts(att, VT32, O32, Sbufs[t % nbuf], Mbufs[t % nbuf], i * RB + 128 * qb, g, offr)
                f = per[t]
                if order == "skew":
                    for x in a: x()
                    for y in b: y()
                    for z in f: z()
                elif order == "inter":
                    for k in range(4):
                        a[k](); b[k]()
                        if k < len(f): f[k]()
                    for z in f[4:]: z()
                elif order == "inter2":
                    for k in range(4):
                        if k < len(f): f[k]()
                        a[k](); b[k]()
                    for z in f[4:]: z()
                elif order == "inter3":
                    for k in range(4):
                        a[k]()
                        if k % 2 == 0 and k // 2 < len(f): f[k // 2]()
                        b[k]()
                    for z in f[2:]: z()
            if post_fn is not None:
                post_fn(i)
            return c
        lax.fori_loop(0, NB, body, 0, unroll=unroll)

    def kernel(xa_h, wqkva_h, woa_h, xb_h, wqkvb_h, wob_h, out_h,
               XA, XB, WQA, WQB, WOA, WOB, OUT,
               QA, KA, VA, OA, QB, KB, VB, OB,
               biasB, biasA, sem_x, sem_w, sem_o, *bufs):
        Mbufs = bufs[:nbuf]
        Sbufs = bufs[nbuf:]
        NB0 = S // RB0

        def cp_xb(i):
            return pltpu.make_async_copy(xb_h.at[pl.ds(i * RB0, RB0)], XB.at[pl.ds(i * RB0, RB0)], sem_x.at[i])

        def cp_w(src, dst, c0, c1, k):
            return pltpu.make_async_copy(src.at[:, c0:c1], dst.at[:, c0:c1], sem_w.at[k])

        wq_b = cp_w(wqkvb_h, WQB, 0, 1024, 0)
        wkv_b = cp_w(wqkvb_h, WQB, 1024, 3072, 1)
        x_a = pltpu.make_async_copy(xa_h, XA, sem_w.at[2])
        w_a = cp_w(wqkva_h, WQA, 0, 3072, 3)
        wo_b = pltpu.make_async_copy(wob_h, WOB, sem_w.at[4])
        wo_a = pltpu.make_async_copy(woa_h, WOA, sem_w.at[5])

        def cp_out(i, br):
            return pltpu.make_async_copy(
                OUT.at[pl.ds(i * RB, RB), pl.ds(br * 1024, 1024)],
                out_h.at[pl.ds(i * RB, RB), pl.ds(br * 1024, 1024)], sem_o.at[br * NB + i])

        cp_xb(0).start()
        wq_b.start()

        zk = jnp.zeros((PAD // 2, D), u32)
        KA[0:PAD // 2, :] = zk
        KB[0:PAD // 2, :] = zk
        zv = jnp.zeros((D // 2, PAD), u32)
        VA[:, 0:PAD] = zv
        VB[:, 0:PAD] = zv
        r = lax.broadcasted_iota(i32, (32, 128), 0)
        jq = lax.broadcasted_iota(i32, (32, 128), 1) % 32
        biasB[0:32, :] = jnp.where(r > jq, 0.0, NEG).astype(f32)
        biasB[32:64, :] = jnp.where(r <= jq, 0.0, NEG).astype(f32)
        r = lax.broadcasted_iota(i32, (48, 128), 0)
        jq = lax.broadcasted_iota(i32, (48, 128), 1) % 32
        rel = 16 + jq - r
        biasA[...] = jnp.where((rel >= 0) & (rel <= 14) & (rel % 2 == 0), 0.0, NEG).astype(f32)

        wq_b.wait()
        cp_xb(0).wait()
        for i in range(1, NB0):
            cp_xb(i).start()

        def p0a(i, c):
            @pl.when(i > 0)
            def _():
                cp_xb(i).wait()

            @pl.when(i == 1)
            def _():
                wkv_b.start()
            for n in range(8):
                qkv_piece(XB, WQB, i * RB0, RB0, n, QB, KB, VB)
            return c
        lax.fori_loop(0, NB0, p0a, 0)

        wkv_b.wait()
        x_a.start()
        w_a.start()

        def p0b(i, c):
            @pl.when(i == NB0 // 2)
            def _():
                wo_b.start()
                wo_a.start()
            for n in range(8, 24):
                qkv_piece(XB, WQB, i * RB0, RB0, n, QB, KB, VB)
            return c
        lax.fori_loop(0, NB0, p0b, 0)

        x_a.wait()
        w_a.wait()
        attn_loop(ATT_B, QB, KB, VB, OB, biasB, Sbufs, Mbufs,
                  lambda i: [functools.partial(qkv_piece, XA, WQA, i * RB, RB, n, QA, KA, VA) for n in range(24)])

        wo_b.wait()
        wo_a.wait()
        attn_loop(ATT_A, QA, KA, VA, OA, biasA, Sbufs, Mbufs,
                  lambda i: [functools.partial(out_piece, OB, WOB, OUT, i * RB, RB, n, 1024) for n in range(1024 // opw)],
                  post_fn=lambda i: cp_out(i, 1).start())

        def p3(i, c):
            for n in range(1024 // opw):
                out_piece(OA, WOA, OUT, i * RB, RB, n, 0)
            cp_out(i, 0).start()
            return c
        lax.fori_loop(0, NB, p3, 0)

        def pw(i, c):
            cp_out(i, 0).wait()
            cp_out(i, 1).wait()
            return c
        lax.fori_loop(0, NB, pw, 0)

    def fn(A_x, A_wqkv, A_wo, B_x, B_wqkv, B_wo):
        xa = A_x.reshape(S, D)
        xb = B_x.reshape(S, D)
        any_spec = pl.BlockSpec(memory_space=pl.ANY)
        scratch = [
            pltpu.VMEM((S, D), bf16), pltpu.VMEM((S, D), bf16),
            pltpu.VMEM((D, 3 * D), bf16), pltpu.VMEM((D, 3 * D), bf16),
            pltpu.VMEM((D, D), bf16), pltpu.VMEM((D, D), bf16),
            pltpu.VMEM((S, 2 * D), bf16),
        ]
        for _ in range(2):
            scratch += [pltpu.VMEM((S // 2, D), u32), pltpu.VMEM(((S + PAD) // 2, D), u32),
                        pltpu.VMEM((D // 2, S + PAD), u32), pltpu.VMEM((S // 2, D), u32)]
        scratch += [pltpu.VMEM((64, 128), f32), pltpu.VMEM((48, 128), f32),
                    pltpu.SemaphoreType.DMA((S // RB0,)), pltpu.SemaphoreType.DMA((6,)),
                    pltpu.SemaphoreType.DMA((2 * NB,))]
        scratch += [pltpu.VMEM((8, 512), f32)] * nbuf
        scratch += [pltpu.VMEM((288, 512), f32)] * nbuf
        out = pl.pallas_call(
            kernel,
            out_shape=jax.ShapeDtypeStruct((S, 2 * D), bf16),
            in_specs=[any_spec] * 6,
            out_specs=any_spec,
            scratch_shapes=scratch,
            compiler_params=pltpu.CompilerParams(vmem_limit_bytes=100 * 2**20),
        )(xa, A_wqkv, A_wo, xb, B_wqkv, B_wo)
        return out.reshape(1, S, 2 * D)

    return jax.jit(fn)


_fn = build()


@jax.jit
def pallas_concat_heads__sliding_local_dilated__sliding_block__prompt_kernel(
    A_x: jax.Array,
    A_wqkv: jax.Array,
    A_wo: jax.Array,
    B_x: jax.Array,
    B_wqkv: jax.Array,
    B_wo: jax.Array,
):
    return _fn(A_x, A_wqkv, A_wo, B_x, B_wqkv, B_wo)
```

```python
import functools
import math

import numpy as np
import jax
import jax.numpy as jnp
from jax import lax
from jax.experimental import pallas as pl
from jax.experimental.pallas import tpu as pltpu

S, D = 2048, 1024
H, DH = 32, 32
PAD = 256
NEG = -1e30
CQ = float(DH ** -0.5 * math.log2(math.e))
bf16, f32, u32, i32 = jnp.bfloat16, jnp.float32, jnp.uint32, jnp.int32


def u2b(x):
    return pltpu.bitcast(x, bf16)


def b2u(x):
    return pltpu.bitcast(x, u32)


def packi(p):
    n = p.shape[0]
    return jnp.concatenate(
        [pltpu.pack_elementwise([p[16 * j:16 * j + 8], p[16 * j + 8:16 * j + 16]], packed_dtype=bf16)
         for j in range(n // 16)], axis=0)


def mo(x, m):
    return pl.multiple_of(x, m)


class _Null:
    def __enter__(self):
        return None

    def __exit__(self, *a):
        return False


class Attn:
    def __init__(self, rows, win0, vwin0, vwidth):
        self.R = rows
        self.win0 = win0
        self.vwin0 = vwin0
        self.vwidth = vwidth
        self.NS = rows // 16
        self.NT = self.NS + 6
        self.lead = (win0 - vwin0) // 16


ATT_B = Attn(288, -256, -256, 384)
ATT_A = Attn(48, -16, -128, 256)


def build(scopes=False, only=None, headB=0, tailB=0, headA=0, tailA=0, forder=tuple(range(24)), wpack=True, padq2=128, ks3d=False, padks=128, fuseB=False, padq=0, padx=0, padl=0, flags=None, strong=0, partial_k=False, depthA=(2, 1), depthB=(2, 1), nsmA=1, nsmB=4, orderA="rrfabc", orderB="rrfabc", RB=256, RB0=512, order="inter2", early="sel", opw=256, unroll=1, nbuf=4, debug=False):
    NB = S // RB

    def so(x):
        return x if strong else pl.multiple_of(x, 8)
    def scope(name):
        return jax.named_scope(name) if scopes else _Null()

    def qkv_piece(X, W, r0, nrows, n, Q32, K32, VT32, packed=False):
        c0 = n * 128
        if packed:
            x = u2b(X[pl.ds(mo(r0 // 2, 8), nrows // 2), 0:D])
            w = u2b(W[:, c0:c0 + 128])
        else:
            x = X[pl.ds(mo(r0, 16), nrows), 0:D]
            w = W[:, c0:c0 + 128]
        r = jnp.dot(x, w, preferred_element_type=f32)
        g = n % 8
        lanes = slice(g * 128, (g + 1) * 128)
        if n < 8:
            Q32.bitcast(bf16)[pl.ds(mo(r0, 16), nrows), lanes] = (r * CQ).astype(bf16)
        elif n < 16:
            K32.bitcast(bf16)[pl.ds(mo(r0 + PAD, 16), nrows), lanes] = r.astype(bf16)
        else:
            vt = u2b(packi(r)).T
            VT32.bitcast(bf16)[lanes, pl.ds(mo(r0 + PAD, 128), nrows)] = vt

    def out_piece(O32, WO, OUT, r0, nrows, n, col0):
        o = u2b(O32[pl.ds(mo(r0 // 2, 8), nrows // 2), 0:D])
        r = jnp.dot(o, WO[:, n * opw:(n + 1) * opw], preferred_element_type=f32)
        OUT[pl.ds(mo(r0, 16), nrows), col0 + n * opw:col0 + (n + 1) * opw] = r.astype(bf16)

    def qk_unit(att, Q32, K32, bias, Sb, Mb, q32, q0, g, s, off):
        lanes = slice(g * 128, (g + 1) * 128)
        lane = lax.broadcasted_iota(i32, (16, 128), 1)
        Qblk = Q32[pl.ds(mo(q32 + 16 * s, 8), 16), lanes]
        zero = jnp.zeros((16, 128), u32)
        Qm = u2b(jnp.concatenate([jnp.where(lane // 32 == h, Qblk, zero) for h in range(4)], axis=0))
        k32 = q32 + (PAD + 32 * s + att.win0) // 2
        Kw = u2b(K32[pl.ds(mo(k32, 8), att.R // 2), lanes])
        St = lax.dot_general(Kw, Qm, (((1,), (1,)), ((), ())), preferred_element_type=f32)
        pieces = []
        if att is ATT_B:
            kpos = q0 + 32 * s - 256
            for i8 in range(9):
                x = St[32 * i8:32 * i8 + 32]
                if i8 == 0:
                    x = x + bias[0:32, :]
                elif i8 == 8:
                    x = x + bias[32:64, :]
                if i8 < 8 and early == "sel":
                    x = jnp.where(kpos + 32 * i8 >= 0, x, NEG)
                pieces.append((32 * i8, x))
        else:
            x0 = St[0:16] + bias[0:16, :]
            if s == 0 and early == "sel":
                x0 = jnp.where(q0 > 0, x0, NEG)
            pieces.append((0, x0))
            pieces.append((16, St[16:48] + bias[16:48, :]))
        mx = None
        for (r0, x) in pieces:
            n = x.shape[0]
            Sb[pl.ds(so(off + r0), n), s * 128:(s + 1) * 128] = x
            y = jnp.max(x.reshape(n // 8, 8, 128), axis=0)
            mx = y if mx is None else jnp.maximum(mx, y)
        Mb[:, s * 128:(s + 1) * 128] = jnp.broadcast_to(jnp.max(mx, axis=0, keepdims=True), (8, 128))

    KSR = 2208

    def qk_sh_parts(Q32, KS, bias, Sb, Mb, q32, q0, g, off):
        lanes = slice(g * 128, (g + 1) * 128)
        lane = lax.broadcasted_iota(i32, (16, 128), 1)
        zero = jnp.zeros((16, 128), u32)
        st = {}

        def one(h):
            if h == 0:
                Qt = Q32[pl.ds(mo(q32, 8), 64), lanes]
                st["R"] = [Qt] + [pltpu.roll(Qt, 32 * t, axis=1) for t in (1, 2, 3)]
            Qm = u2b(jnp.concatenate(
                [jnp.where(lane // 32 == s, st["R"][(s - h) % 4][16 * s:16 * (s + 1)], zero) for s in range(4)], axis=0))
            Kw = u2b(KS[4 * g + h, pl.ds(mo(q32, 8), 144), :]) if ks3d else u2b(KS[pl.ds(mo(q32, 8), 144), (4 * g + h) * 128:(4 * g + h + 1) * 128])
            St = lax.dot_general(Kw, Qm, (((1,), (1,)), ((), ())), preferred_element_type=f32)
            slot32 = (lax.broadcasted_iota(i32, (1, 128), 1) // 32) * 32
            pieces = []
            for i8 in range(9):
                x = St[32 * i8:32 * i8 + 32]
                if i8 == 0:
                    x = x + bias[0:32, :]
                elif i8 == 8:
                    x = x + bias[32:64, :]
                if i8 < 8 and early == "sel":
                    x = jnp.where(q0 + slot32 + (32 * i8 - 256) >= 0, x, NEG)
                pieces.append((32 * i8, x))
            mx = None
            for (r0, x) in pieces:
                n = x.shape[0]
                Sb[pl.ds(so(off + r0), n), h * 128:(h + 1) * 128] = x
                y = jnp.max(x.reshape(n // 8, 8, 128), axis=0)
                mx = y if mx is None else jnp.maximum(mx, y)
            Mb[:, h * 128:(h + 1) * 128] = jnp.broadcast_to(jnp.max(mx, axis=0, keepdims=True), (8, 128))
        return [functools.partial(one, h) for h in range(4)]

    def sm_sh_parts(Sb, Mb, Tb, Lb, offr, offw):
        lane8 = lax.broadcasted_iota(i32, (8, 128), 1)
        zero8 = jnp.zeros((8, 128), u32)

        def blk(s):
            return lane8 // 32 == s

        def one(h):
            m = Mb[:, h * 128:(h + 1) * 128]
            pu = []
            l = None
            for a in range(24):
                if a < 18:
                    x = Sb[pl.ds(so(offr + 16 * a), 16), h * 128:(h + 1) * 128]
                    p0 = jnp.exp2(x[0:8] - m)
                    p1 = jnp.exp2(x[8:16] - m)
                    ps = p0 + p1
                    l = ps if l is None else l + ps
                    pu.append(pltpu.pack_elementwise([p0, p1], packed_dtype=bf16))
                cur = None
                for s in range(4):
                    src = a - 2 * s
                    if 0 <= src < 18:
                        cur = jnp.where(blk(s), pu[src], zero8 if cur is None else cur)
                Tb[pl.ds(so(offw + 8 * a), 8), h * 128:(h + 1) * 128] = cur
            ls = jnp.broadcast_to(jnp.sum(l, axis=0, keepdims=True), (8, 128))
            Lb[pl.ds(so(offw), 8), h * 128:(h + 1) * 128] = 1.0 / ls
        return [functools.partial(one, h) for h in range(4)]

    def smpv_sh_parts(VT32, O32, Sb, Mb, q0, g, offr):
        lane8 = lax.broadcasted_iota(i32, (8, 128), 1)
        zero8 = jnp.zeros((8, 128), u32)
        ots = []

        def blk(s):
            return lane8 // 32 == s

        def one(h):
            m = Mb[:, h * 128:(h + 1) * 128]
            pu = []
            T = []
            l = None
            for a in range(24):
                if a < 18:
                    x = Sb[pl.ds(so(offr + 16 * a), 16), h * 128:(h + 1) * 128]
                    p0 = jnp.exp2(x[0:8] - m)
                    p1 = jnp.exp2(x[8:16] - m)
                    ps = p0 + p1
                    l = ps if l is None else l + ps
                    pu.append(pltpu.pack_elementwise([p0, p1], packed_dtype=bf16))
                cur = None
                for s in range(4):
                    src = a - 2 * s
                    if 0 <= src < 18:
                        cur = jnp.where(blk(s), pu[src], zero8 if cur is None else cur)
                T.append(cur)
            ls = jnp.broadcast_to(jnp.sum(l, axis=0, keepdims=True), (8, 128))
            inv = 1.0 / ls
            f32row = (g * 128 + h * 32) // 2
            Vt = u2b(VT32[f32row:f32row + 16, pl.ds(mo(q0, 128), 384)])
            ot = jnp.dot(Vt, u2b(jnp.concatenate(T, axis=0)), preferred_element_type=f32)
            ots.append(ot * jnp.concatenate([inv] * 4, axis=0))
            if h == 3:
                OTg = jnp.concatenate(ots, axis=0).astype(bf16)
                O32.bitcast(bf16)[pl.ds(mo(q0, 128), 128), g * 128:(g + 1) * 128] = OTg.T
        return [functools.partial(one, h) for h in range(4)]

    def build_ks(K32, KS, b0, nb):
        lane8 = lax.broadcasted_iota(i32, (8, 128), 1)
        thunks = []

        def one(g):
            R = {}

            def rot(b):
                if b not in R:
                    v = K32[pl.ds(mo((b0 + b) * 8, 8), 8), g * 128:(g + 1) * 128]
                    R[b] = [v] + [pltpu.roll(v, 32 * t, axis=1) for t in (1, 2, 3)]
                return R[b]
            for b in range(nb):
                for h in range(4):
                    cur = rot(b)[(0 - h) % 4]
                    for s in range(1, 4):
                        cur = jnp.where(lane8 // 32 == s, rot(b + 2 * s)[(s - h) % 4], cur)
                    if ks3d:
                        KS[4 * g + h, pl.ds(mo((b0 + b) * 8, 8), 8), :] = cur
                    else:
                        KS[pl.ds(mo((b0 + b) * 8, 8), 8), (4 * g + h) * 128:(4 * g + h + 1) * 128] = cur
        return [functools.partial(one, g) for g in range(8)]

    def sm_parts(att, Sb, Mb, Tb, Lb, offr, offw, nparts):
        st = {"l": [None] * 4}
        lane8 = lax.broadcasted_iota(i32, (8, 128), 1)
        zero8 = jnp.zeros((8, 128), u32)

        def blk(s):
            return lane8 // 32 == s

        def do_a(a):
            rots = {}
            for s in range(4):
                src = a - 2 * s
                if 0 <= src < att.NS:
                    m = Mb[:, s * 128:(s + 1) * 128]
                    x = Sb[pl.ds(so(offr + 16 * src), 16), s * 128:(s + 1) * 128]
                    p0 = jnp.exp2(x[0:8] - m)
                    p1 = jnp.exp2(x[8:16] - m)
                    ps = p0 + p1
                    st["l"][s] = ps if st["l"][s] is None else st["l"][s] + ps
                    pu = pltpu.pack_elementwise([p0, p1], packed_dtype=bf16)
                    rots[s] = [pu] + [pltpu.roll(pu, 32 * t, axis=1) for t in (1, 2, 3)]
            for h in range(4):
                cur = None
                for s in rots:
                    v = rots[s][(s - h) % 4]
                    cur = jnp.where(blk(s), v, zero8 if cur is None else cur)
                Tb[pl.ds(so(offw + 8 * a), 8), h * 128:(h + 1) * 128] = cur

        def finish():
            lred = []
            for s in range(4):
                ls = jnp.broadcast_to(jnp.sum(st["l"][s], axis=0, keepdims=True), (8, 128))
                lred.append([ls] + [pltpu.roll(ls, 32 * t, axis=1) for t in (1, 2, 3)])
            for h in range(4):
                lh = None
                for s in range(4):
                    v = lred[s][(s - h) % 4]
                    lh = v if lh is None else jnp.where(blk(s), v, lh)
                Lb[pl.ds(so(offw), 8), h * 128:(h + 1) * 128] = 1.0 / lh

        nt = att.NT
        bounds = [(nt * k) // nparts for k in range(nparts + 1)]

        def part(k):
            for a in range(bounds[k], bounds[k + 1]):
                do_a(a)
            if k == nparts - 1:
                finish()
        return [functools.partial(part, k) for k in range(nparts)]

    def pv_parts(att, VT32, O32, Tb, Lb, q0, g, offr):
        ots = []

        def one(h):
            T = Tb[pl.ds(so(offr), 8 * att.NT), h * 128:(h + 1) * 128]
            if att.lead:
                if partial_k:
                    Th = u2b(T)
                else:
                    Th = u2b(jnp.concatenate([jnp.zeros((8 * att.lead, 128), u32), T], axis=0))
            else:
                Th = u2b(T)
            f32row = (g * 128 + h * 32) // 2
            Vt = u2b(VT32[f32row:f32row + 16, pl.ds(mo(q0 + PAD + att.vwin0, 128), att.vwidth)])
            if att.lead and partial_k:
                Vt = Vt[:, 16 * att.lead:]
            ot = jnp.dot(Vt, Th, preferred_element_type=f32)
            inv = Lb[pl.ds(so(offr), 8), h * 128:(h + 1) * 128]
            ots.append(ot * jnp.concatenate([inv] * 4, axis=0))
            if h == 3:
                OTg = jnp.concatenate(ots, axis=0).astype(bf16)
                O32.bitcast(bf16)[pl.ds(mo(q0, 128), 128), g * 128:(g + 1) * 128] = OTg.T
        return [functools.partial(one, h) for h in range(4)]

    def attn_loop(att, Q32, K32, VT32, O32, bias, Sbufs, Mbufs, Tbufs, Lbufs, fillers_fn, pre_fn=None, post_fn=None):
        nqb = RB // 128
        steps = [(qb, g) for qb in range(nqb) for g in range(8)]
        ns = len(steps)
        depth = depthB if att is ATT_B else depthA

        def locate(i, t):
            if t >= ns:
                i2 = jnp.minimum(i + 1, NB - 1)
                qb, g = steps[t - ns]
            else:
                i2 = i
                qb, g = steps[t]
            return i2, qb, g

        def qk_parts(i, t, offw):
            i2, qb, g = locate(i, t)
            q32 = i2 * (RB // 2) + 64 * qb
            q0 = i2 * RB + 128 * qb
            slot = t % nbuf
            if att is ATT_B:
                return qk_sh_parts(Q32, K32, bias, Sbufs[slot], Mbufs[slot], q32, q0, g, offw)
            return [functools.partial(qk_unit, att, Q32, K32, bias, Sbufs[slot], Mbufs[slot], q32, q0, g, s, offw)
                    for s in range(4)]

        def sm_p(t, offr, offw):
            if att is ATT_B:
                return sm_sh_parts(Sbufs[t % nbuf], Mbufs[t % nbuf], Tbufs[t % nbuf], Lbufs[t % nbuf], offr, offw)
            return sm_parts(att, Sbufs[t % nbuf], Mbufs[t % nbuf], Tbufs[t % nbuf], Lbufs[t % nbuf], offr, offw,
                            nsmB if att is ATT_B else nsmA)

        for t in range(depth[0]):
            for f in qk_parts(0, t, 0):
                f()
        fused = fuseB and att is ATT_B
        for t in range(depth[1]):
            if not fused:
                for f in sm_p(t, 0, 0):
                    f()

        def body(i, c):
            o1 = i >> 8
            o2 = i >> 9
            o3 = i >> 10
            o4 = i >> 11
            if strong:
                o1, o2, o3, o4 = [pl.multiple_of(o * strong, strong) for o in (o1, o2, o3, o4)]
            if pre_fn is not None:
                pre_fn(i)
            fl = fillers_fn(i)
            nf = len(fl)
            nhead, ntail = (headB, tailB) if att is ATT_B else (headA, tailA)
            per = [fl[nhead + ((nf - nhead - ntail) * t) // ns:nhead + ((nf - nhead - ntail) * (t + 1)) // ns] for t in range(ns)]
            for x in fl[:nhead]:
                x()
            for t in range(ns):
                a = qk_parts(i, t + depth[0], o1)
                qb, g = steps[t]
                if fused:
                    b = []
                    c_ = smpv_sh_parts(VT32, O32, Sbufs[t % nbuf], Mbufs[t % nbuf], i * RB + 128 * qb, g, o2)
                else:
                    b = sm_p(t + depth[1], o2, o3)
                    c_ = pv_parts(att, VT32, O32, Tbufs[t % nbuf], Lbufs[t % nbuf], i * RB + 128 * qb, g, o4)
                f = list(per[t])
                ordr = orderB if att is ATT_B else orderA
                if ordr == "spread":
                    items = [((k + 0.5) / len(L), j, x) for j, L in enumerate((f, a, b, c_)) if L for k, x in enumerate(L)]
                    for _, _, x in sorted(items, key=lambda it: (it[0], it[1])): x()
                else:
                    L = {"f": f, "a": a, "b": b, "c": c_}
                    n = max(len(v) for v in L.values())
                    if ordr.startswith("rr"):
                        for k in range(n):
                            for ch in ordr[2:]:
                                if k < len(L[ch]): L[ch][k]()
                    else:
                        for ch in ordr:
                            for x in L[ch]: x()
            for x in fl[nf - ntail:]:
                x()
            if post_fn is not None:
                post_fn(i)
            return c
        with scope("attn_B" if att is ATT_B else "attn_A"):
            lax.fori_loop(0, NB, body, 0, unroll=unroll)

    def kernel(xa_h, wqkva_h, woa_h, xb_h, wqkvb_h, wob_h, out_h,
               XA, XB, WQA, WQB, WOA, WOB, OUT,
               QA, KA, VA, OA, QB, KB, VB, OB,
               XA32, WQA32, KS, biasB, biasA, sem_x, sem_w, sem_o, sem_xa, sem_wa, *bufs):
        Mbufs = bufs[:nbuf]
        Sbufs = bufs[nbuf:2 * nbuf]
        Tbufs = bufs[2 * nbuf:3 * nbuf]
        Lbufs = bufs[3 * nbuf:4 * nbuf]
        NB0 = S // RB0

        def cp_xb(i):
            return pltpu.make_async_copy(xb_h.at[pl.ds(i * RB0, RB0)], XB.at[pl.ds(i * RB0, RB0), 0:D], sem_x.at[i])

        def cp_w(src, dst, c0, c1, k):
            return pltpu.make_async_copy(src.at[:, c0:c1], dst.at[:, c0:c1], sem_w.at[k])

        wq_b = cp_w(wqkvb_h, WQB, 1024, 2048, 0)
        wkv_b = cp_w(wqkvb_h, WQB, 0, 1024, 1)
        wkv_b2 = cp_w(wqkvb_h, WQB, 2048, 3072, 6)
        def cp_xa(i):
            return pltpu.make_async_copy(xa_h.at[pl.ds(i * RB0, RB0)], XA.at[pl.ds(i * RB0, RB0), 0:D], sem_xa.at[i])

        def cp_wa(i):
            wr = D // NB0
            return pltpu.make_async_copy(wqkva_h.at[pl.ds(i * wr, wr)], WQA.at[pl.ds(i * wr, wr), 0:3 * D], sem_wa.at[i])
        wo_b = pltpu.make_async_copy(wob_h, WOB.at[:, 0:D], sem_w.at[4])
        wo_a = pltpu.make_async_copy(woa_h, WOA.at[:, 0:D], sem_w.at[5])

        def cp_out(i, br):
            return pltpu.make_async_copy(
                OUT.at[pl.ds(i * RB, RB), pl.ds(br * 1024, 1024)],
                out_h.at[pl.ds(i * RB, RB), pl.ds(br * 1024, 1024)], sem_o.at[br * NB + i])

        cp_xb(0).start()
        wq_b.start()

        zk = jnp.zeros((PAD // 2, D), u32)
        KA[0:PAD // 2, 0:D] = zk
        KB[0:PAD // 2, 0:D] = zk
        zv = jnp.zeros((D // 2, PAD), u32)
        VA[:, 0:PAD] = zv
        VB[:, 0:PAD] = zv
        r = lax.broadcasted_iota(i32, (32, 128), 0)
        jq = lax.broadcasted_iota(i32, (32, 128), 1) % 32
        biasB[0:32, :] = jnp.where(r > jq, 0.0, NEG).astype(f32)
        biasB[32:64, :] = jnp.where(r <= jq, 0.0, NEG).astype(f32)
        r = lax.broadcasted_iota(i32, (48, 128), 0)
        jq = lax.broadcasted_iota(i32, (48, 128), 1) % 32
        rel = 16 + jq - r
        biasA[...] = jnp.where((rel >= 0) & (rel <= 14) & (rel % 2 == 0), 0.0, NEG).astype(f32)

        with scope("wait0"):
            wq_b.wait()
            cp_xb(0).wait()
        for i in range(1, NB0):
            cp_xb(i).start()

        def p0a(i, c):
            @pl.when(i > 0)
            def _():
                cp_xb(i).wait()

            @pl.when(i == 1)
            def _():
                wkv_b.start()
                wkv_b2.start()

            @pl.when(i == 2)
            def _():
                for j in range(NB0 // 2):
                    cp_xa(j).start()
                    cp_wa(j).start()

            @pl.when(i == NB0 - 1)
            def _():
                for j in range(NB0 // 2, NB0):
                    cp_xa(j).start()
                    cp_wa(j).start()
            for n in range(8, 16):
                qkv_piece(XB, WQB, i * RB0, RB0, n, QB, KB, VB)
            return c
        if only in (None, 'p0a'):
          with scope('p0a'):
            lax.fori_loop(0, NB0, p0a, 0)

        with scope("wait_wkv"):
            wkv_b.wait()
            wkv_b2.wait()
        def p0b(i, c):
            cp_xa(i).wait()
            cp_wa(i).wait()

            @pl.when(i == 0)
            def _():
                wo_b.start()
                wo_a.start()
            nbk = (KSR // 16 + NB0 - 1) // NB0
            ks = build_ks(KB, KS, jnp.minimum(i * nbk, KSR // 16 - nbk), nbk)
            pcs = list(range(0, 8)) + list(range(16, 24))
            for j, n in enumerate(pcs):
                qkv_piece(XB, WQB, i * RB0, RB0, n, QB, KB, VB)
                if j % 2 == 1:
                    ks[j // 2]()
                elif wpack:
                    jj = j // 2
                    rr = RB0 // 8
                    XA32.bitcast(bf16)[pl.ds(mo(i * RB0 + jj * rr, 16), rr), 0:D] = XA[pl.ds(mo(i * RB0 + jj * rr, 16), rr), 0:D]
                    wr = D // NB0 // 8
                    WQA32.bitcast(bf16)[pl.ds(mo(i * (D // NB0) + jj * wr, 16), wr), 0:3 * D] = WQA[pl.ds(mo(i * (D // NB0) + jj * wr, 16), wr), 0:3 * D]
            return c
        if only in (None, 'p0b'):
          with scope('p0b'):
            lax.fori_loop(0, NB0, p0b, 0)

        if only in (None, 'B'):
          attn_loop(ATT_B, QB, KS, VB, OB, biasB, Sbufs, Mbufs, Tbufs, Lbufs,
                  lambda i: [functools.partial(qkv_piece, XA32 if wpack else XA, WQA32 if wpack else WQA, i * RB, RB, n, QA, KA, VA, wpack) for n in forder])

        with scope("wait_wo"):
            wo_b.wait()
            wo_a.wait()
        if only in (None, 'A'):
          attn_loop(ATT_A, QA, KA, VA, OA, biasA, Sbufs, Mbufs, Tbufs, Lbufs,
                  lambda i: [functools.partial(out_piece, OB, WOB, OUT, i * RB, RB, n, 1024) for n in range(1024 // opw)],
                  post_fn=lambda i: cp_out(i, 1).start())

        def p3(i, c):
            for n in range(1024 // opw):
                out_piece(OA, WOA, OUT, i * RB, RB, n, 0)
            cp_out(i, 0).start()
            return c
        if only in (None, 'p3'):
          with scope('p3'):
            lax.fori_loop(0, NB, p3, 0)

        if only is not None:
            OUT[0:16, 0:128] = u2b(QA[0:8, 0:128] ^ KA[128:136, 0:128] ^ VA[0:8, 256:384] ^ OB[0:8, 0:128] ^ OA[0:8, 0:128]
                                   ^ QB[0:8, 0:128] ^ KB[128:136, 0:128] ^ VB[0:8, 256:384] ^ XA32[0:8, 0:128] ^ WQA32[0:8, 0:128] ^ KS[0:8, 0:128])

        def pw(i, c):
            cp_out(i, 0).wait()
            cp_out(i, 1).wait()
            return c
        with scope('tail'):
            lax.fori_loop(0, NB, pw, 0)

    def fn(A_x, A_wqkv, A_wo, B_x, B_wqkv, B_wo):
        xa = A_x.reshape(S, D)
        xb = B_x.reshape(S, D)
        any_spec = pl.BlockSpec(memory_space=pl.ANY)
        scratch = [
            pltpu.VMEM((S, D + padx), bf16), pltpu.VMEM((S, D + padx), bf16),
            pltpu.VMEM((D, 3 * D + padx), bf16), pltpu.VMEM((D, 3 * D + padx), bf16),
            pltpu.VMEM((D, D + padx), bf16), pltpu.VMEM((D, D + padx), bf16),
            pltpu.VMEM((S, 2 * D), bf16),
        ]
        for _ in range(2):
            scratch += [pltpu.VMEM((S // 2, D + padq), u32), pltpu.VMEM(((S + PAD) // 2, D + padq), u32),
                        pltpu.VMEM((D // 2, S + PAD), u32), pltpu.VMEM((S // 2, D + padq), u32)]
        scratch += [pltpu.VMEM((S // 2, D + padq2), u32), pltpu.VMEM((D // 2, 3 * D + padq2), u32)]
        scratch += [(pltpu.VMEM((32, KSR // 2, 128), u32) if ks3d else pltpu.VMEM((KSR // 2, 4096 + padks), u32)), pltpu.VMEM((64, 128), f32), pltpu.VMEM((48, 128), f32),
                    pltpu.SemaphoreType.DMA((S // RB0,)), pltpu.SemaphoreType.DMA((7,)),
                    pltpu.SemaphoreType.DMA((2 * NB,)), pltpu.SemaphoreType.DMA((S // RB0,)), pltpu.SemaphoreType.DMA((S // RB0,))]
        scratch += [pltpu.VMEM((8, 512), f32)] * nbuf
        scratch += [pltpu.VMEM((288, 512 + padl), f32)] * nbuf
        scratch += [pltpu.VMEM((192, 512 + padl), u32)] * nbuf
        scratch += [pltpu.VMEM((8, 512), f32)] * nbuf
        out = pl.pallas_call(
            kernel,
            out_shape=jax.ShapeDtypeStruct((S, 2 * D), bf16),
            in_specs=[any_spec] * 6,
            out_specs=any_spec,
            scratch_shapes=scratch,
            compiler_params=pltpu.CompilerParams(vmem_limit_bytes=110 * 2**20, flags=flags),
        )(xa, A_wqkv, A_wo, xb, B_wqkv, B_wo)
        return out.reshape(1, S, 2 * D)

    return jax.jit(fn)


_fn = build(opw=128, padl=128, padx=128, fuseB=True, depthB=(2,0), orderB="rrcfa", forder=tuple(x for p in zip(range(8,16),range(16,24),range(0,8)) for x in p), headB=1, tailB=1, orderA="fabc", depthA=(3,1), partial_k=True, headA=1, tailA=1)


@jax.jit
def pallas_concat_heads__sliding_local_dilated__sliding_block__prompt_kernel(
    A_x: jax.Array,
    A_wqkv: jax.Array,
    A_wo: jax.Array,
    B_x: jax.Array,
    B_wqkv: jax.Array,
    B_wo: jax.Array,
):
    return _fn(A_x, A_wqkv, A_wo, B_x, B_wqkv, B_wo)
```

```python
import functools
import math

import numpy as np
import jax
import jax.numpy as jnp
from jax import lax
from jax.experimental import pallas as pl
from jax.experimental.pallas import tpu as pltpu

S, D = 2048, 1024
H, DH = 32, 32
PAD = 256
NEG = -1e30
CQ = float(DH ** -0.5 * math.log2(math.e))
bf16, f32, u32, i32 = jnp.bfloat16, jnp.float32, jnp.uint32, jnp.int32


def u2b(x):
    return pltpu.bitcast(x, bf16)


def b2u(x):
    return pltpu.bitcast(x, u32)


def packi(p):
    n = p.shape[0]
    return jnp.concatenate(
        [pltpu.pack_elementwise([p[16 * j:16 * j + 8], p[16 * j + 8:16 * j + 16]], packed_dtype=bf16)
         for j in range(n // 16)], axis=0)


def mo(x, m):
    return pl.multiple_of(x, m)


class _Null:
    def __enter__(self):
        return None

    def __exit__(self, *a):
        return False


class Attn:
    def __init__(self, rows, win0, vwin0, vwidth):
        self.R = rows
        self.win0 = win0
        self.vwin0 = vwin0
        self.vwidth = vwidth
        self.NS = rows // 16
        self.NT = self.NS + 6
        self.lead = (win0 - vwin0) // 16


ATT_B = Attn(288, -256, -256, 384)
ATT_A = Attn(48, -16, -128, 256)


def build(scopes=False, ahead=1, nwk=4, xstart=1, only=None, headB=0, tailB=0, headA=0, tailA=0, forder=tuple(range(24)), wpack=True, padq2=128, ks3d=False, padks=128, fuseB=False, padq=0, padx=0, padl=0, flags=None, strong=0, partial_k=False, depthA=(2, 1), depthB=(2, 1), nsmA=1, nsmB=4, orderA="rrfabc", orderB="rrfabc", RB=256, RB0=512, order="inter2", early="sel", opw=256, unroll=1, nbuf=4, debug=False):
    NB = S // RB

    def so(x):
        return x if strong else pl.multiple_of(x, 8)
    def scope(name):
        return jax.named_scope(name) if scopes else _Null()

    def qkv_piece(X, W, r0, nrows, n, Q32, K32, VT32, packed=False):
        c0 = n * 128
        if packed:
            x = u2b(X[pl.ds(mo(r0 // 2, 8), nrows // 2), 0:D])
            w = u2b(W[:, c0:c0 + 128])
        else:
            x = X[pl.ds(mo(r0, 16), nrows), 0:D]
            w = W[:, c0:c0 + 128]
        r = jnp.dot(x, w, preferred_element_type=f32)
        g = n % 8
        lanes = slice(g * 128, (g + 1) * 128)
        if n < 8:
            Q32.bitcast(bf16)[pl.ds(mo(r0, 16), nrows), lanes] = (r * CQ).astype(bf16)
        elif n < 16:
            K32.bitcast(bf16)[pl.ds(mo(r0 + PAD, 16), nrows), lanes] = r.astype(bf16)
        else:
            vt = u2b(packi(r)).T
            VT32.bitcast(bf16)[lanes, pl.ds(mo(r0 + PAD, 128), nrows)] = vt

    def out_piece(O32, WO, OUT, r0, nrows, n, col0):
        o = u2b(O32[pl.ds(mo(r0 // 2, 8), nrows // 2), 0:D])
        r = jnp.dot(o, WO[:, n * opw:(n + 1) * opw], preferred_element_type=f32)
        OUT[pl.ds(mo(r0, 16), nrows), col0 + n * opw:col0 + (n + 1) * opw] = r.astype(bf16)

    def qk_unit(att, Q32, K32, bias, Sb, Mb, q32, q0, g, s, off):
        lanes = slice(g * 128, (g + 1) * 128)
        lane = lax.broadcasted_iota(i32, (16, 128), 1)
        Qblk = Q32[pl.ds(mo(q32 + 16 * s, 8), 16), lanes]
        zero = jnp.zeros((16, 128), u32)
        Qm = u2b(jnp.concatenate([jnp.where(lane // 32 == h, Qblk, zero) for h in range(4)], axis=0))
        k32 = q32 + (PAD + 32 * s + att.win0) // 2
        Kw = u2b(K32[pl.ds(mo(k32, 8), att.R // 2), lanes])
        St = lax.dot_general(Kw, Qm, (((1,), (1,)), ((), ())), preferred_element_type=f32)
        pieces = []
        if att is ATT_B:
            kpos = q0 + 32 * s - 256
            for i8 in range(9):
                x = St[32 * i8:32 * i8 + 32]
                if i8 == 0:
                    x = x + bias[0:32, :]
                elif i8 == 8:
                    x = x + bias[32:64, :]
                if i8 < 8 and early == "sel":
                    x = jnp.where(kpos + 32 * i8 >= 0, x, NEG)
                pieces.append((32 * i8, x))
        else:
            x0 = St[0:16] + bias[0:16, :]
            if s == 0 and early == "sel":
                x0 = jnp.where(q0 > 0, x0, NEG)
            pieces.append((0, x0))
            pieces.append((16, St[16:48] + bias[16:48, :]))
        mx = None
        for (r0, x) in pieces:
            n = x.shape[0]
            Sb[pl.ds(so(off + r0), n), s * 128:(s + 1) * 128] = x
            y = jnp.max(x.reshape(n // 8, 8, 128), axis=0)
            mx = y if mx is None else jnp.maximum(mx, y)
        Mb[:, s * 128:(s + 1) * 128] = jnp.broadcast_to(jnp.max(mx, axis=0, keepdims=True), (8, 128))

    KSR = 2208

    def qk_sh_parts(Q32, KS, bias, Sb, Mb, q32, q0, g, off):
        lanes = slice(g * 128, (g + 1) * 128)
        lane = lax.broadcasted_iota(i32, (16, 128), 1)
        zero = jnp.zeros((16, 128), u32)
        st = {}

        def one(h):
            if h == 0:
                Qt = Q32[pl.ds(mo(q32, 8), 64), lanes]
                st["R"] = [Qt] + [pltpu.roll(Qt, 32 * t, axis=1) for t in (1, 2, 3)]
            Qm = u2b(jnp.concatenate(
                [jnp.where(lane // 32 == s, st["R"][(s - h) % 4][16 * s:16 * (s + 1)], zero) for s in range(4)], axis=0))
            Kw = u2b(KS[4 * g + h, pl.ds(mo(q32, 8), 144), :]) if ks3d else u2b(KS[pl.ds(mo(q32, 8), 144), (4 * g + h) * 128:(4 * g + h + 1) * 128])
            St = lax.dot_general(Kw, Qm, (((1,), (1,)), ((), ())), preferred_element_type=f32)
            slot32 = (lax.broadcasted_iota(i32, (1, 128), 1) // 32) * 32
            pieces = []
            for i8 in range(9):
                x = St[32 * i8:32 * i8 + 32]
                if i8 == 0:
                    x = x + bias[0:32, :]
                elif i8 == 8:
                    x = x + bias[32:64, :]
                if i8 < 8 and early == "sel":
                    x = jnp.where(q0 + slot32 + (32 * i8 - 256) >= 0, x, NEG)
                pieces.append((32 * i8, x))
            mx = None
            for (r0, x) in pieces:
                n = x.shape[0]
                Sb[pl.ds(so(off + r0), n), h * 128:(h + 1) * 128] = x
                y = jnp.max(x.reshape(n // 8, 8, 128), axis=0)
                mx = y if mx is None else jnp.maximum(mx, y)
            Mb[:, h * 128:(h + 1) * 128] = jnp.broadcast_to(jnp.max(mx, axis=0, keepdims=True), (8, 128))
        return [functools.partial(one, h) for h in range(4)]

    def sm_sh_parts(Sb, Mb, Tb, Lb, offr, offw):
        lane8 = lax.broadcasted_iota(i32, (8, 128), 1)
        zero8 = jnp.zeros((8, 128), u32)

        def blk(s):
            return lane8 // 32 == s

        def one(h):
            m = Mb[:, h * 128:(h + 1) * 128]
            pu = []
            l = None
            for a in range(24):
                if a < 18:
                    x = Sb[pl.ds(so(offr + 16 * a), 16), h * 128:(h + 1) * 128]
                    p0 = jnp.exp2(x[0:8] - m)
                    p1 = jnp.exp2(x[8:16] - m)
                    ps = p0 + p1
                    l = ps if l is None else l + ps
                    pu.append(pltpu.pack_elementwise([p0, p1], packed_dtype=bf16))
                cur = None
                for s in range(4):
                    src = a - 2 * s
                    if 0 <= src < 18:
                        cur = jnp.where(blk(s), pu[src], zero8 if cur is None else cur)
                Tb[pl.ds(so(offw + 8 * a), 8), h * 128:(h + 1) * 128] = cur
            ls = jnp.broadcast_to(jnp.sum(l, axis=0, keepdims=True), (8, 128))
            Lb[pl.ds(so(offw), 8), h * 128:(h + 1) * 128] = 1.0 / ls
        return [functools.partial(one, h) for h in range(4)]

    def smpv_sh_parts(VT32, O32, Sb, Mb, q0, g, offr):
        lane8 = lax.broadcasted_iota(i32, (8, 128), 1)
        zero8 = jnp.zeros((8, 128), u32)
        ots = []

        def blk(s):
            return lane8 // 32 == s

        def one(h):
            m = Mb[:, h * 128:(h + 1) * 128]
            pu = []
            T = []
            l = None
            for a in range(24):
                if a < 18:
                    x = Sb[pl.ds(so(offr + 16 * a), 16), h * 128:(h + 1) * 128]
                    p0 = jnp.exp2(x[0:8] - m)
                    p1 = jnp.exp2(x[8:16] - m)
                    ps = p0 + p1
                    l = ps if l is None else l + ps
                    pu.append(pltpu.pack_elementwise([p0, p1], packed_dtype=bf16))
                cur = None
                for s in range(4):
                    src = a - 2 * s
                    if 0 <= src < 18:
                        cur = jnp.where(blk(s), pu[src], zero8 if cur is None else cur)
                T.append(cur)
            ls = jnp.broadcast_to(jnp.sum(l, axis=0, keepdims=True), (8, 128))
            inv = 1.0 / ls
            f32row = (g * 128 + h * 32) // 2
            Vt = u2b(VT32[f32row:f32row + 16, pl.ds(mo(q0, 128), 384)])
            ot = jnp.dot(Vt, u2b(jnp.concatenate(T, axis=0)), preferred_element_type=f32)
            ots.append(ot * jnp.concatenate([inv] * 4, axis=0))
            if h == 3:
                OTg = jnp.concatenate(ots, axis=0).astype(bf16)
                O32.bitcast(bf16)[pl.ds(mo(q0, 128), 128), g * 128:(g + 1) * 128] = OTg.T
        return [functools.partial(one, h) for h in range(4)]

    def build_ks(K32, KS, b0, nb):
        lane8 = lax.broadcasted_iota(i32, (8, 128), 1)
        thunks = []

        def one(g):
            R = {}

            def rot(b):
                if b not in R:
                    v = K32[pl.ds(mo((b0 + b) * 8, 8), 8), g * 128:(g + 1) * 128]
                    R[b] = [v] + [pltpu.roll(v, 32 * t, axis=1) for t in (1, 2, 3)]
                return R[b]
            for b in range(nb):
                for h in range(4):
                    cur = rot(b)[(0 - h) % 4]
                    for s in range(1, 4):
                        cur = jnp.where(lane8 // 32 == s, rot(b + 2 * s)[(s - h) % 4], cur)
                    if ks3d:
                        KS[4 * g + h, pl.ds(mo((b0 + b) * 8, 8), 8), :] = cur
                    else:
                        KS[pl.ds(mo((b0 + b) * 8, 8), 8), (4 * g + h) * 128:(4 * g + h + 1) * 128] = cur
        return [functools.partial(one, g) for g in range(8)]

    def sm_parts(att, Sb, Mb, Tb, Lb, offr, offw, nparts):
        st = {"l": [None] * 4}
        lane8 = lax.broadcasted_iota(i32, (8, 128), 1)
        zero8 = jnp.zeros((8, 128), u32)

        def blk(s):
            return lane8 // 32 == s

        def do_a(a):
            rots = {}
            for s in range(4):
                src = a - 2 * s
                if 0 <= src < att.NS:
                    m = Mb[:, s * 128:(s + 1) * 128]
                    x = Sb[pl.ds(so(offr + 16 * src), 16), s * 128:(s + 1) * 128]
                    p0 = jnp.exp2(x[0:8] - m)
                    p1 = jnp.exp2(x[8:16] - m)
                    ps = p0 + p1
                    st["l"][s] = ps if st["l"][s] is None else st["l"][s] + ps
                    pu = pltpu.pack_elementwise([p0, p1], packed_dtype=bf16)
                    rots[s] = [pu] + [pltpu.roll(pu, 32 * t, axis=1) for t in (1, 2, 3)]
            for h in range(4):
                cur = None
                for s in rots:
                    v = rots[s][(s - h) % 4]
                    cur = jnp.where(blk(s), v, zero8 if cur is None else cur)
                Tb[pl.ds(so(offw + 8 * a), 8), h * 128:(h + 1) * 128] = cur

        def finish():
            lred = []
            for s in range(4):
                ls = jnp.broadcast_to(jnp.sum(st["l"][s], axis=0, keepdims=True), (8, 128))
                lred.append([ls] + [pltpu.roll(ls, 32 * t, axis=1) for t in (1, 2, 3)])
            for h in range(4):
                lh = None
                for s in range(4):
                    v = lred[s][(s - h) % 4]
                    lh = v if lh is None else jnp.where(blk(s), v, lh)
                Lb[pl.ds(so(offw), 8), h * 128:(h + 1) * 128] = 1.0 / lh

        nt = att.NT
        bounds = [(nt * k) // nparts for k in range(nparts + 1)]

        def part(k):
            for a in range(bounds[k], bounds[k + 1]):
                do_a(a)
            if k == nparts - 1:
                finish()
        return [functools.partial(part, k) for k in range(nparts)]

    def pv_parts(att, VT32, O32, Tb, Lb, q0, g, offr):
        ots = []

        def one(h):
            T = Tb[pl.ds(so(offr), 8 * att.NT), h * 128:(h + 1) * 128]
            if att.lead:
                if partial_k:
                    Th = u2b(T)
                else:
                    Th = u2b(jnp.concatenate([jnp.zeros((8 * att.lead, 128), u32), T], axis=0))
            else:
                Th = u2b(T)
            f32row = (g * 128 + h * 32) // 2
            Vt = u2b(VT32[f32row:f32row + 16, pl.ds(mo(q0 + PAD + att.vwin0, 128), att.vwidth)])
            if att.lead and partial_k:
                Vt = Vt[:, 16 * att.lead:]
            ot = jnp.dot(Vt, Th, preferred_element_type=f32)
            inv = Lb[pl.ds(so(offr), 8), h * 128:(h + 1) * 128]
            ots.append(ot * jnp.concatenate([inv] * 4, axis=0))
            if h == 3:
                OTg = jnp.concatenate(ots, axis=0).astype(bf16)
                O32.bitcast(bf16)[pl.ds(mo(q0, 128), 128), g * 128:(g + 1) * 128] = OTg.T
        return [functools.partial(one, h) for h in range(4)]

    def attn_loop(att, Q32, K32, VT32, O32, bias, Sbufs, Mbufs, Tbufs, Lbufs, fillers_fn, pre_fn=None, post_fn=None):
        nqb = RB // 128
        steps = [(qb, g) for qb in range(nqb) for g in range(8)]
        ns = len(steps)
        depth = depthB if att is ATT_B else depthA

        def locate(i, t):
            if t >= ns:
                i2 = jnp.minimum(i + 1, NB - 1)
                qb, g = steps[t - ns]
            else:
                i2 = i
                qb, g = steps[t]
            return i2, qb, g

        def qk_parts(i, t, offw):
            i2, qb, g = locate(i, t)
            q32 = i2 * (RB // 2) + 64 * qb
            q0 = i2 * RB + 128 * qb
            slot = t % nbuf
            if att is ATT_B:
                return qk_sh_parts(Q32, K32, bias, Sbufs[slot], Mbufs[slot], q32, q0, g, offw)
            return [functools.partial(qk_unit, att, Q32, K32, bias, Sbufs[slot], Mbufs[slot], q32, q0, g, s, offw)
                    for s in range(4)]

        def sm_p(t, offr, offw):
            if att is ATT_B:
                return sm_sh_parts(Sbufs[t % nbuf], Mbufs[t % nbuf], Tbufs[t % nbuf], Lbufs[t % nbuf], offr, offw)
            return sm_parts(att, Sbufs[t % nbuf], Mbufs[t % nbuf], Tbufs[t % nbuf], Lbufs[t % nbuf], offr, offw,
                            nsmB if att is ATT_B else nsmA)

        for t in range(depth[0]):
            for f in qk_parts(0, t, 0):
                f()
        fused = fuseB and att is ATT_B
        for t in range(depth[1]):
            if not fused:
                for f in sm_p(t, 0, 0):
                    f()

        def body(i, c):
            o1 = i >> 8
            o2 = i >> 9
            o3 = i >> 10
            o4 = i >> 11
            if strong:
                o1, o2, o3, o4 = [pl.multiple_of(o * strong, strong) for o in (o1, o2, o3, o4)]
            if pre_fn is not None:
                pre_fn(i)
            fl = fillers_fn(i)
            nf = len(fl)
            nhead, ntail = (headB, tailB) if att is ATT_B else (headA, tailA)
            per = [fl[nhead + ((nf - nhead - ntail) * t) // ns:nhead + ((nf - nhead - ntail) * (t + 1)) // ns] for t in range(ns)]
            for x in fl[:nhead]:
                x()
            for t in range(ns):
                a = qk_parts(i, t + depth[0], o1)
                qb, g = steps[t]
                if fused:
                    b = []
                    c_ = smpv_sh_parts(VT32, O32, Sbufs[t % nbuf], Mbufs[t % nbuf], i * RB + 128 * qb, g, o2)
                else:
                    b = sm_p(t + depth[1], o2, o3)
                    c_ = pv_parts(att, VT32, O32, Tbufs[t % nbuf], Lbufs[t % nbuf], i * RB + 128 * qb, g, o4)
                f = list(per[t])
                ordr = orderB if att is ATT_B else orderA
                if ordr == "spread":
                    items = [((k + 0.5) / len(L), j, x) for j, L in enumerate((f, a, b, c_)) if L for k, x in enumerate(L)]
                    for _, _, x in sorted(items, key=lambda it: (it[0], it[1])): x()
                else:
                    L = {"f": f, "a": a, "b": b, "c": c_}
                    n = max(len(v) for v in L.values())
                    if ordr.startswith("rr"):
                        for k in range(n):
                            for ch in ordr[2:]:
                                if k < len(L[ch]): L[ch][k]()
                    else:
                        for ch in ordr:
                            for x in L[ch]: x()
            for x in fl[nf - ntail:]:
                x()
            if post_fn is not None:
                post_fn(i)
            return c
        with scope("attn_B" if att is ATT_B else "attn_A"):
            lax.fori_loop(0, NB, body, 0, unroll=unroll)

    def kernel(xa_h, wqkva_h, woa_h, xb_h, wqkvb_h, wob_h, out_h,
               XA, XB, WQA, WQB, WOA, WOB, OUT,
               QA, KA, VA, OA, QB, KB, VB, OB,
               XA32, WQA32, KS, biasB, biasA, sem_x, sem_w, sem_o, sem_xa, sem_wa, *bufs):
        Mbufs = bufs[:nbuf]
        Sbufs = bufs[nbuf:2 * nbuf]
        Tbufs = bufs[2 * nbuf:3 * nbuf]
        Lbufs = bufs[3 * nbuf:4 * nbuf]
        NB0 = S // RB0

        def cp_xb(i):
            return pltpu.make_async_copy(xb_h.at[pl.ds(i * RB0, RB0)], XB.at[pl.ds(i * RB0, RB0), 0:D], sem_x.at[i])

        def cp_w(src, dst, c0, c1, k):
            return pltpu.make_async_copy(src.at[:, c0:c1], dst.at[:, c0:c1], sem_w.at[k])

        wk_b = [cp_w(wqkvb_h, WQB, 1024 + j * (1024 // nwk), 1024 + (j + 1) * (1024 // nwk), (0, 2, 3, 5)[j] if False else 7 + j) for j in range(nwk)]
        wkv_b = cp_w(wqkvb_h, WQB, 0, 1024, 1)
        wkv_b2 = cp_w(wqkvb_h, WQB, 2048, 3072, 6)
        def cp_xa(i):
            return pltpu.make_async_copy(xa_h.at[pl.ds(i * RB0, RB0)], XA.at[pl.ds(i * RB0, RB0), 0:D], sem_xa.at[i])

        def cp_wa(i):
            wr = D // NB0
            return pltpu.make_async_copy(wqkva_h.at[pl.ds(i * wr, wr)], WQA.at[pl.ds(i * wr, wr), 0:3 * D], sem_wa.at[i])
        wo_b = pltpu.make_async_copy(wob_h, WOB.at[:, 0:D], sem_w.at[4])
        wo_a = pltpu.make_async_copy(woa_h, WOA.at[:, 0:D], sem_w.at[5])

        def cp_out(i, br):
            return pltpu.make_async_copy(
                OUT.at[pl.ds(i * RB, RB), pl.ds(br * 1024, 1024)],
                out_h.at[pl.ds(i * RB, RB), pl.ds(br * 1024, 1024)], sem_o.at[br * NB + i])

        cp_xb(0).start()
        wk_b[0].start()

        zk = jnp.zeros((PAD // 2, D), u32)
        KA[0:PAD // 2, 0:D] = zk
        KB[0:PAD // 2, 0:D] = zk
        zv = jnp.zeros((D // 2, PAD), u32)
        VA[:, 0:PAD] = zv
        VB[:, 0:PAD] = zv
        r = lax.broadcasted_iota(i32, (32, 128), 0)
        jq = lax.broadcasted_iota(i32, (32, 128), 1) % 32
        biasB[0:32, :] = jnp.where(r > jq, 0.0, NEG).astype(f32)
        biasB[32:64, :] = jnp.where(r <= jq, 0.0, NEG).astype(f32)
        r = lax.broadcasted_iota(i32, (48, 128), 0)
        jq = lax.broadcasted_iota(i32, (48, 128), 1) % 32
        rel = 16 + jq - r
        biasA[...] = jnp.where((rel >= 0) & (rel <= 14) & (rel % 2 == 0), 0.0, NEG).astype(f32)

        with scope("wait0"):
            wk_b[0].wait()
            cp_xb(0).wait()
        with scope("p0a0"):
            for j in range(nwk):
                if j > 0:
                    wk_b[j].wait()
                if j == 0:
                    for jj in range(1, min(nwk, 1 + ahead)):
                        wk_b[jj].start()
                elif j + ahead < nwk:
                    wk_b[j + ahead].start()
                if j == xstart:
                    cp_xb(1).start()
                if j == nwk - 1:
                    for i in range(2, NB0):
                        cp_xb(i).start()
                for n in range(8 + j * (8 // nwk), 8 + (j + 1) * (8 // nwk)):
                    qkv_piece(XB, WQB, 0, RB0, n, QB, KB, VB)

        def p0a(i, c):
            cp_xb(i).wait()

            @pl.when(i == 1)
            def _():
                wkv_b.start()
                wkv_b2.start()

            @pl.when(i == 2)
            def _():
                for j in range(NB0 // 2):
                    cp_xa(j).start()
                    cp_wa(j).start()

            @pl.when(i == NB0 - 1)
            def _():
                for j in range(NB0 // 2, NB0):
                    cp_xa(j).start()
                    cp_wa(j).start()
            for n in range(8, 16):
                qkv_piece(XB, WQB, i * RB0, RB0, n, QB, KB, VB)
            return c
        if only in (None, 'p0a'):
          with scope('p0a'):
            lax.fori_loop(1, NB0, p0a, 0)

        with scope("wait_wkv"):
            wkv_b.wait()
            wkv_b2.wait()
        def p0b(i, c):
            cp_xa(i).wait()
            cp_wa(i).wait()

            @pl.when(i == 0)
            def _():
                wo_b.start()
                wo_a.start()
            nbk = (KSR // 16 + NB0 - 1) // NB0
            ks = build_ks(KB, KS, jnp.minimum(i * nbk, KSR // 16 - nbk), nbk)
            pcs = list(range(0, 8)) + list(range(16, 24))
            for j, n in enumerate(pcs):
                qkv_piece(XB, WQB, i * RB0, RB0, n, QB, KB, VB)
                if j % 2 == 1:
                    ks[j // 2]()
                elif wpack:
                    jj = j // 2
                    rr = RB0 // 8
                    XA32.bitcast(bf16)[pl.ds(mo(i * RB0 + jj * rr, 16), rr), 0:D] = XA[pl.ds(mo(i * RB0 + jj * rr, 16), rr), 0:D]
                    wr = D // NB0 // 8
                    WQA32.bitcast(bf16)[pl.ds(mo(i * (D // NB0) + jj * wr, 16), wr), 0:3 * D] = WQA[pl.ds(mo(i * (D // NB0) + jj * wr, 16), wr), 0:3 * D]
            return c
        if only in (None, 'p0b'):
          with scope('p0b'):
            lax.fori_loop(0, NB0, p0b, 0)

        if only in (None, 'B'):
          attn_loop(ATT_B, QB, KS, VB, OB, biasB, Sbufs, Mbufs, Tbufs, Lbufs,
                  lambda i: [functools.partial(qkv_piece, XA32 if wpack else XA, WQA32 if wpack else WQA, i * RB, RB, n, QA, KA, VA, wpack) for n in forder])

        with scope("wait_wo"):
            wo_b.wait()
            wo_a.wait()
        if only in (None, 'A'):
          attn_loop(ATT_A, QA, KA, VA, OA, biasA, Sbufs, Mbufs, Tbufs, Lbufs,
                  lambda i: [functools.partial(out_piece, OB, WOB, OUT, i * RB, RB, n, 1024) for n in range(1024 // opw)],
                  post_fn=lambda i: cp_out(i, 1).start())

        def p3(i, c):
            for n in range(1024 // opw):
                out_piece(OA, WOA, OUT, i * RB, RB, n, 0)
            cp_out(i, 0).start()
            return c
        if only in (None, 'p3'):
          with scope('p3'):
            lax.fori_loop(0, NB, p3, 0)

        if only is not None:
            OUT[0:16, 0:128] = u2b(QA[0:8, 0:128] ^ KA[128:136, 0:128] ^ VA[0:8, 256:384] ^ OB[0:8, 0:128] ^ OA[0:8, 0:128]
                                   ^ QB[0:8, 0:128] ^ KB[128:136, 0:128] ^ VB[0:8, 256:384] ^ XA32[0:8, 0:128] ^ WQA32[0:8, 0:128] ^ KS[0:8, 0:128])

        def pw(i, c):
            cp_out(i, 0).wait()
            cp_out(i, 1).wait()
            return c
        with scope('tail'):
            lax.fori_loop(0, NB, pw, 0)

    def fn(A_x, A_wqkv, A_wo, B_x, B_wqkv, B_wo):
        xa = A_x.reshape(S, D)
        xb = B_x.reshape(S, D)
        any_spec = pl.BlockSpec(memory_space=pl.ANY)
        scratch = [
            pltpu.VMEM((S, D + padx), bf16), pltpu.VMEM((S, D + padx), bf16),
            pltpu.VMEM((D, 3 * D + padx), bf16), pltpu.VMEM((D, 3 * D + padx), bf16),
            pltpu.VMEM((D, D + padx), bf16), pltpu.VMEM((D, D + padx), bf16),
            pltpu.VMEM((S, 2 * D), bf16),
        ]
        for _ in range(2):
            scratch += [pltpu.VMEM((S // 2, D + padq), u32), pltpu.VMEM(((S + PAD) // 2, D + padq), u32),
                        pltpu.VMEM((D // 2, S + PAD), u32), pltpu.VMEM((S // 2, D + padq), u32)]
        scratch += [pltpu.VMEM((S // 2, D + padq2), u32), pltpu.VMEM((D // 2, 3 * D + padq2), u32)]
        scratch += [(pltpu.VMEM((32, KSR // 2, 128), u32) if ks3d else pltpu.VMEM((KSR // 2, 4096 + padks), u32)), pltpu.VMEM((64, 128), f32), pltpu.VMEM((48, 128), f32),
                    pltpu.SemaphoreType.DMA((S // RB0,)), pltpu.SemaphoreType.DMA((7 + nwk,)),
                    pltpu.SemaphoreType.DMA((2 * NB,)), pltpu.SemaphoreType.DMA((S // RB0,)), pltpu.SemaphoreType.DMA((S // RB0,))]
        scratch += [pltpu.VMEM((8, 512), f32)] * nbuf
        scratch += [pltpu.VMEM((288, 512 + padl), f32)] * nbuf
        scratch += [pltpu.VMEM((192, 512 + padl), u32)] * nbuf
        scratch += [pltpu.VMEM((8, 512), f32)] * nbuf
        out = pl.pallas_call(
            kernel,
            out_shape=jax.ShapeDtypeStruct((S, 2 * D), bf16),
            in_specs=[any_spec] * 6,
            out_specs=any_spec,
            scratch_shapes=scratch,
            compiler_params=pltpu.CompilerParams(vmem_limit_bytes=110 * 2**20, flags=flags),
        )(xa, A_wqkv, A_wo, xb, B_wqkv, B_wo)
        return out.reshape(1, S, 2 * D)

    return jax.jit(fn)


_fn = build(opw=128, padl=128, padx=128, fuseB=True, depthB=(2,0), orderB="rrcfa", forder=tuple(x for p in zip(range(8,16),range(16,24),range(0,8)) for x in p), headB=1, tailB=1, orderA="fabc", depthA=(3,1), partial_k=True, headA=1, tailA=1, nwk=4, xstart=2)


@jax.jit
def pallas_concat_heads__sliding_local_dilated__sliding_block__prompt_kernel(
    A_x: jax.Array,
    A_wqkv: jax.Array,
    A_wo: jax.Array,
    B_x: jax.Array,
    B_wqkv: jax.Array,
    B_wo: jax.Array,
):
    return _fn(A_x, A_wqkv, A_wo, B_x, B_wqkv, B_wo)
```

```python
import functools
import math

import jax
import jax.numpy as jnp
from jax import lax
import jax.experimental.pallas as pl
import jax.experimental.pallas.tpu as pltpu

S, D = 2048, 1024
DH = 32
PAD = 256
RB0 = 512
RB = 256
NB0, NB = S // RB0, S // RB
NBUF = 4
KSR = 2208
NWK = 4
LP = 128
NEG = -1e30
CQ = float(DH ** -0.5 * math.log2(math.e))
bf16, f32, u32, i32 = jnp.bfloat16, jnp.float32, jnp.uint32, jnp.int32
P = functools.partial


def u2b(x):
    return pltpu.bitcast(x, bf16)


def mo(x, m):
    return pl.multiple_of(x, m)


def pack2(p0, p1):
    return pltpu.pack_elementwise([p0, p1], packed_dtype=bf16)


def qkv_piece(X, W, r0, nrows, n, Q32, K32, VT32, packed):
    if packed:
        x = u2b(X[pl.ds(mo(r0 // 2, 8), nrows // 2), 0:D])
        w = u2b(W[:, n * 128:(n + 1) * 128])
    else:
        x = X[pl.ds(mo(r0, 16), nrows), 0:D]
        w = W[:, n * 128:(n + 1) * 128]
    r = jnp.dot(x, w, preferred_element_type=f32)
    lanes = slice((n % 8) * 128, (n % 8 + 1) * 128)
    if n < 8:
        Q32.bitcast(bf16)[pl.ds(mo(r0, 16), nrows), lanes] = (r * CQ).astype(bf16)
    elif n < 16:
        K32.bitcast(bf16)[pl.ds(mo(r0 + PAD, 16), nrows), lanes] = r.astype(bf16)
    else:
        vp = jnp.concatenate([pack2(r[16 * j:16 * j + 8], r[16 * j + 8:16 * j + 16])
                              for j in range(nrows // 16)], axis=0)
        VT32.bitcast(bf16)[lanes, pl.ds(mo(r0 + PAD, 128), nrows)] = u2b(vp).T


def out_piece(O32, WO, OUT, r0, n, col0):
    o = u2b(O32[pl.ds(mo(r0 // 2, 8), RB // 2), 0:D])
    r = jnp.dot(o, WO[:, n * 128:(n + 1) * 128], preferred_element_type=f32)
    OUT[pl.ds(mo(r0, 16), RB), col0 + n * 128:col0 + (n + 1) * 128] = r.astype(bf16)


def build_ks(K32, KS, b0, nb):
    lane = lax.broadcasted_iota(i32, (8, 128), 1)

    def one(g):
        rots = {}

        def rot(b):
            if b not in rots:
                v = K32[pl.ds(mo((b0 + b) * 8, 8), 8), g * 128:(g + 1) * 128]
                rots[b] = [v] + [pltpu.roll(v, 32 * t, axis=1) for t in (1, 2, 3)]
            return rots[b]
        for b in range(nb):
            for h in range(4):
                cur = rot(b)[(0 - h) % 4]
                for s in range(1, 4):
                    cur = jnp.where(lane // 32 == s, rot(b + 2 * s)[(s - h) % 4], cur)
                KS[pl.ds(mo((b0 + b) * 8, 8), 8), (4 * g + h) * 128:(4 * g + h + 1) * 128] = cur
    return [P(one, g) for g in range(8)]


def store_scores(pieces, Sb, Mb, off, c):
    cols = slice(c * 128, (c + 1) * 128)
    mx = None
    for r0, x in pieces:
        n = x.shape[0]
        Sb[pl.ds(mo(off + r0, 8), n), cols] = x
        y = jnp.max(x.reshape(n // 8, 8, 128), axis=0)
        mx = y if mx is None else jnp.maximum(mx, y)
    Mb[:, cols] = jnp.broadcast_to(jnp.max(mx, axis=0, keepdims=True), (8, 128))


def store_heads(ots, O32, q0, g):
    ot = jnp.concatenate(ots, axis=0).astype(bf16)
    O32.bitcast(bf16)[pl.ds(mo(q0, 128), 128), g * 128:(g + 1) * 128] = ot.T


def b_qk(Q32, KS, bias, Sb, Mb, q32, q0, g, off):
    lane = lax.broadcasted_iota(i32, (16, 128), 1)
    zero = jnp.zeros((16, 128), u32)
    st = {}

    def one(h):
        if h == 0:
            qt = Q32[pl.ds(mo(q32, 8), 64), g * 128:(g + 1) * 128]
            st["R"] = [qt] + [pltpu.roll(qt, 32 * t, axis=1) for t in (1, 2, 3)]
        qm = u2b(jnp.concatenate(
            [jnp.where(lane // 32 == s, st["R"][(s - h) % 4][16 * s:16 * (s + 1)], zero) for s in range(4)], axis=0))
        kw = u2b(KS[pl.ds(mo(q32, 8), 144), (4 * g + h) * 128:(4 * g + h + 1) * 128])
        sc = lax.dot_general(kw, qm, (((1,), (1,)), ((), ())), preferred_element_type=f32)
        slot32 = (lax.broadcasted_iota(i32, (1, 128), 1) // 32) * 32
        pieces = []
        for i8 in range(9):
            x = sc[32 * i8:32 * i8 + 32]
            if i8 == 0:
                x = x + bias[0:32, :]
            elif i8 == 8:
                x = x + bias[32:64, :]
            if i8 < 8:
                x = jnp.where(q0 + slot32 + (32 * i8 - 256) >= 0, x, NEG)
            pieces.append((32 * i8, x))
        store_scores(pieces, Sb, Mb, off, h)
    return [P(one, h) for h in range(4)]


def b_smpv(VT32, O32, Sb, Mb, q0, g, off):
    lane = lax.broadcasted_iota(i32, (8, 128), 1)
    zero = jnp.zeros((8, 128), u32)
    ots = []

    def one(h):
        cols = slice(h * 128, (h + 1) * 128)
        m = Mb[:, cols]
        pu, tiles, l = [], [], None
        for a in range(24):
            if a < 18:
                x = Sb[pl.ds(mo(off + 16 * a, 8), 16), cols]
                p0 = jnp.exp2(x[0:8] - m)
                p1 = jnp.exp2(x[8:16] - m)
                l = p0 + p1 if l is None else l + (p0 + p1)
                pu.append(pack2(p0, p1))
            cur = None
            for s in range(4):
                if 0 <= a - 2 * s < 18:
                    cur = jnp.where(lane // 32 == s, pu[a - 2 * s], zero if cur is None else cur)
            tiles.append(cur)
        inv = 1.0 / jnp.broadcast_to(jnp.sum(l, axis=0, keepdims=True), (8, 128))
        fr = (g * 128 + h * 32) // 2
        vt = u2b(VT32[fr:fr + 16, pl.ds(mo(q0, 128), 384)])
        ot = jnp.dot(vt, u2b(jnp.concatenate(tiles, axis=0)), preferred_element_type=f32)
        ots.append(ot * jnp.concatenate([inv] * 4, axis=0))
        if h == 3:
            store_heads(ots, O32, q0, g)
    return [P(one, h) for h in range(4)]


def a_qk(Q32, K32, bias, Sb, Mb, q32, q0, g, off):
    lanes = slice(g * 128, (g + 1) * 128)
    lane = lax.broadcasted_iota(i32, (16, 128), 1)
    zero = jnp.zeros((16, 128), u32)

    def one(s):
        qb = Q32[pl.ds(mo(q32 + 16 * s, 8), 16), lanes]
        qm = u2b(jnp.concatenate([jnp.where(lane // 32 == h, qb, zero) for h in range(4)], axis=0))
        kw = u2b(K32[pl.ds(mo(q32 + (PAD + 32 * s - 16) // 2, 8), 24), lanes])
        sc = lax.dot_general(kw, qm, (((1,), (1,)), ((), ())), preferred_element_type=f32)
        x0 = sc[0:16] + bias[0:16, :]
        if s == 0:
            x0 = jnp.where(q0 > 0, x0, NEG)
        store_scores([(0, x0), (16, sc[16:48] + bias[16:48, :])], Sb, Mb, off, s)
    return [P(one, s) for s in range(4)]


def a_sm(Sb, Mb, Tb, Lb, offr, offw):
    lane = lax.broadcasted_iota(i32, (8, 128), 1)
    zero = jnp.zeros((8, 128), u32)

    def rolls(x):
        return [x] + [pltpu.roll(x, 32 * t, axis=1) for t in (1, 2, 3)]

    def run():
        l = [None] * 4
        for a in range(9):
            rots = {}
            for s in range(4):
                if 0 <= a - 2 * s < 3:
                    m = Mb[:, s * 128:(s + 1) * 128]
                    x = Sb[pl.ds(mo(offr + 16 * (a - 2 * s), 8), 16), s * 128:(s + 1) * 128]
                    p0 = jnp.exp2(x[0:8] - m)
                    p1 = jnp.exp2(x[8:16] - m)
                    l[s] = p0 + p1 if l[s] is None else l[s] + (p0 + p1)
                    rots[s] = rolls(pack2(p0, p1))
            for h in range(4):
                cur = None
                for s in rots:
                    cur = jnp.where(lane // 32 == s, rots[s][(s - h) % 4], zero if cur is None else cur)
                Tb[pl.ds(mo(offw + 8 * a, 8), 8), h * 128:(h + 1) * 128] = cur
        lr = [rolls(jnp.broadcast_to(jnp.sum(l[s], axis=0, keepdims=True), (8, 128))) for s in range(4)]
        for h in range(4):
            lh = lr[0][(0 - h) % 4]
            for s in range(1, 4):
                lh = jnp.where(lane // 32 == s, lr[s][(s - h) % 4], lh)
            Lb[pl.ds(mo(offw, 8), 8), h * 128:(h + 1) * 128] = 1.0 / lh
    return [run]


def a_pv(VT32, O32, Tb, Lb, q0, g, off):
    ots = []

    def one(h):
        cols = slice(h * 128, (h + 1) * 128)
        th = u2b(Tb[pl.ds(mo(off, 8), 72), cols])
        fr = (g * 128 + h * 32) // 2
        vt = u2b(VT32[fr:fr + 16, pl.ds(mo(q0 + PAD - 128, 128), 256)])[:, 112:]
        ot = jnp.dot(vt, th, preferred_element_type=f32)
        inv = Lb[pl.ds(mo(off, 8), 8), cols]
        ots.append(ot * jnp.concatenate([inv] * 4, axis=0))
        if h == 3:
            store_heads(ots, O32, q0, g)
    return [P(one, h) for h in range(4)]


def attn_loop(is_b, Q32, K32, VT32, O32, bias, Sb, Mb, Tb, Lb, fillers_fn, post_fn=None):
    steps = [(qb, g) for qb in range(RB // 128) for g in range(8)]
    ns = len(steps)
    dq, ds = (2, 0) if is_b else (3, 1)

    def qk(i, t, off):
        if t >= ns:
            i = jnp.minimum(i + 1, NB - 1)
        qb, g = steps[t % ns]
        return (b_qk if is_b else a_qk)(Q32, K32, bias, Sb[t % NBUF], Mb[t % NBUF],
                                        i * (RB // 2) + 64 * qb, i * RB + 128 * qb, g, off)

    def sm(t, offr, offw):
        return [] if is_b else a_sm(Sb[t % NBUF], Mb[t % NBUF], Tb[t % NBUF], Lb[t % NBUF], offr, offw)

    for t in range(dq):
        for f in qk(0, t, 0):
            f()
    for t in range(ds):
        for f in sm(t, 0, 0):
            f()

    def body(i, c):
        o1, o2, o3, o4 = i >> 8, i >> 9, i >> 10, i >> 11
        fl = fillers_fn(i)
        nf = len(fl) - 2
        fl[0]()
        for t in range(ns):
            qb, g = steps[t]
            q0 = i * RB + 128 * qb
            fs = fl[1 + (nf * t) // ns:1 + (nf * (t + 1)) // ns]
            qs = qk(i, t + dq, o1)
            if is_b:
                pv = b_smpv(VT32, O32, Sb[t % NBUF], Mb[t % NBUF], q0, g, o2)
                for k in range(4):
                    pv[k]()
                    if k < len(fs):
                        fs[k]()
                    qs[k]()
            else:
                ss = sm(t + ds, o2, o3)
                pv = a_pv(VT32, O32, Tb[t % NBUF], Lb[t % NBUF], q0, g, o4)
                for f in fs + qs + ss + pv:
                    f()
        fl[-1]()
        if post_fn is not None:
            post_fn(i)
        return c
    lax.fori_loop(0, NB, body, 0)


def kernel(xa_h, wqa_h, woa_h, xb_h, wqb_h, wob_h, out_h,
           XA, XB, WQA, WQB, WOA, WOB, OUT, QA, KA, VA, OA, QB, KB, VB, OB,
           XA32, WQA32, KS, bias_b, bias_a, sem_x, sem_w, sem_o, sem_xa, sem_wa, *bufs):
    Mb, Sb, Tb, Lb = (bufs[k * NBUF:(k + 1) * NBUF] for k in range(4))

    def cp_xb(i):
        return pltpu.make_async_copy(xb_h.at[pl.ds(i * RB0, RB0)], XB.at[pl.ds(i * RB0, RB0), 0:D], sem_x.at[i])

    def cp_xa(i):
        return pltpu.make_async_copy(xa_h.at[pl.ds(i * RB0, RB0)], XA.at[pl.ds(i * RB0, RB0), 0:D], sem_xa.at[i])

    def cp_wa(i):
        wr = D // NB0
        return pltpu.make_async_copy(wqa_h.at[pl.ds(i * wr, wr)], WQA.at[pl.ds(i * wr, wr), 0:3 * D], sem_wa.at[i])

    def cp_wb(c0, c1, k):
        return pltpu.make_async_copy(wqb_h.at[:, c0:c1], WQB.at[:, c0:c1], sem_w.at[k])

    def cp_out(i, c0, w, k):
        return pltpu.make_async_copy(OUT.at[pl.ds(i * RB, RB), pl.ds(c0, w)],
                                     out_h.at[pl.ds(i * RB, RB), pl.ds(c0, w)], sem_o.at[k])

    wk_b = [cp_wb(D + j * (D // NWK), D + (j + 1) * (D // NWK), j) for j in range(NWK)]
    wq_b, wv_b = cp_wb(0, D, NWK), cp_wb(2 * D, 3 * D, NWK + 1)
    wo_b = pltpu.make_async_copy(wob_h, WOB.at[:, 0:D], sem_w.at[NWK + 2])
    wo_a = pltpu.make_async_copy(woa_h, WOA.at[:, 0:D], sem_w.at[NWK + 3])

    cp_xb(0).start()
    wk_b[0].start()

    zk = jnp.zeros((PAD // 2, D), u32)
    KA[0:PAD // 2, :] = zk
    KB[0:PAD // 2, :] = zk
    zv = jnp.zeros((D // 2, PAD), u32)
    VA[:, 0:PAD] = zv
    VB[:, 0:PAD] = zv
    r = lax.broadcasted_iota(i32, (32, 128), 0)
    jq = lax.broadcasted_iota(i32, (32, 128), 1) % 32
    bias_b[0:32, :] = jnp.where(r > jq, 0.0, NEG).astype(f32)
    bias_b[32:64, :] = jnp.where(r <= jq, 0.0, NEG).astype(f32)
    rel = 16 + lax.broadcasted_iota(i32, (48, 128), 1) % 32 - lax.broadcasted_iota(i32, (48, 128), 0)
    bias_a[...] = jnp.where((rel >= 0) & (rel <= 14) & (rel % 2 == 0), 0.0, NEG).astype(f32)

    cp_xb(0).wait()
    for j in range(NWK):
        wk_b[j].wait()
        if j + 1 < NWK:
            wk_b[j + 1].start()
        if j == 2:
            cp_xb(1).start()
        if j == NWK - 1:
            for i in range(2, NB0):
                cp_xb(i).start()
        for n in range(8 + j * (8 // NWK), 8 + (j + 1) * (8 // NWK)):
            qkv_piece(XB, WQB, 0, RB0, n, QB, KB, VB, False)

    def p0a(i, c):
        cp_xb(i).wait()

        @pl.when(i == 1)
        def _():
            wq_b.start()
            wv_b.start()

        @pl.when(i == 2)
        def _():
            for j in range(NB0 // 2):
                cp_xa(j).start()
                cp_wa(j).start()

        @pl.when(i == NB0 - 1)
        def _():
            for j in range(NB0 // 2, NB0):
                cp_xa(j).start()
                cp_wa(j).start()
        for n in range(8, 16):
            qkv_piece(XB, WQB, i * RB0, RB0, n, QB, KB, VB, False)
        return c
    lax.fori_loop(1, NB0, p0a, 0)

    wq_b.wait()
    wv_b.wait()

    def p0b(i, c):
        cp_xa(i).wait()
        cp_wa(i).wait()

        @pl.when(i == 0)
        def _():
            wo_b.start()
            wo_a.start()
        nbk = (KSR // 16 + NB0 - 1) // NB0
        ks = build_ks(KB, KS, jnp.minimum(i * nbk, KSR // 16 - nbk), nbk)
        for j, n in enumerate(list(range(0, 8)) + list(range(16, 24))):
            qkv_piece(XB, WQB, i * RB0, RB0, n, QB, KB, VB, False)
            if j % 2 == 1:
                ks[j // 2]()
            else:
                xr = pl.ds(mo(i * RB0 + (j // 2) * (RB0 // 8), 16), RB0 // 8)
                XA32.bitcast(bf16)[xr, 0:D] = XA[xr, 0:D]
                wr = pl.ds(mo(i * (D // NB0) + (j // 2) * (D // NB0 // 8), 16), D // NB0 // 8)
                WQA32.bitcast(bf16)[wr, 0:3 * D] = WQA[wr, 0:3 * D]
        return c
    lax.fori_loop(0, NB0, p0b, 0)

    order = [n for g in range(8) for n in (8 + g, 16 + g, g)]
    attn_loop(True, QB, KS, VB, OB, bias_b, Sb, Mb, Tb, Lb,
              lambda i: [P(qkv_piece, XA32, WQA32, i * RB, RB, n, QA, KA, VA, True) for n in order])

    wo_b.wait()
    wo_a.wait()
    attn_loop(False, QA, KA, VA, OA, bias_a, Sb, Mb, Tb, Lb,
              lambda i: [P(out_piece, OB, WOB, OUT, i * RB, n, D) for n in range(8)],
              lambda i: cp_out(i, D, D, 0).start())

    def p3(i, c):
        for n in range(8):
            out_piece(OA, WOA, OUT, i * RB, n, 0)
            cp_out(i, n * 128, 128, 1).start()
        return c
    lax.fori_loop(0, NB, p3, 0)

    def drain(i, c):
        for n in range(8):
            cp_out(i, n * 128, 128, 1).wait()
        cp_out(i, D, D, 0).wait()
        return c
    lax.fori_loop(0, NB, drain, 0)


@jax.jit
def pallas_concat_heads__sliding_local_dilated__sliding_block__prompt_kernel(
    A_x: jax.Array,
    A_wqkv: jax.Array,
    A_wo: jax.Array,
    B_x: jax.Array,
    B_wqkv: jax.Array,
    B_wo: jax.Array,
):
    vm = pltpu.VMEM
    scratch = [vm((S, D + LP), bf16)] * 2 + [vm((D, 3 * D + LP), bf16)] * 2 + [vm((D, D + LP), bf16)] * 2
    scratch += [vm((S, 2 * D), bf16)]
    scratch += [vm((S // 2, D), u32), vm(((S + PAD) // 2, D), u32), vm((D // 2, S + PAD), u32),
                vm((S // 2, D), u32)] * 2
    scratch += [vm((S // 2, D + LP), u32), vm((D // 2, 3 * D + LP), u32), vm((KSR // 2, 32 * 128 + LP), u32),
                vm((64, 128), f32), vm((48, 128), f32)]
    dma = pltpu.SemaphoreType.DMA
    scratch += [dma((NB0,)), dma((NWK + 4,)), dma((2,)), dma((NB0,)), dma((NB0,))]
    scratch += [vm((8, 512), f32)] * NBUF + [vm((288, 512 + LP), f32)] * NBUF
    scratch += [vm((72, 512 + LP), u32)] * NBUF + [vm((8, 512), f32)] * NBUF
    any_spec = pl.BlockSpec(memory_space=pl.ANY)
    out = pl.pallas_call(
        kernel,
        out_shape=jax.ShapeDtypeStruct((S, 2 * D), bf16),
        in_specs=[any_spec] * 6,
        out_specs=any_spec,
        scratch_shapes=scratch,
        compiler_params=pltpu.CompilerParams(vmem_limit_bytes=110 * 2**20),
    )(A_x.reshape(S, D), A_wqkv, A_wo, B_x.reshape(S, D), B_wqkv, B_wo)
    return out.reshape(1, S, 2 * D)
```
